```python
import os as _os
_os.environ.setdefault("JAX_PLATFORMS", "cpu")
import jax
import jax.numpy as jnp

def _softmax(x, axis=-1):
    return jax.nn.softmax(x, axis=axis)
def _gelu(x):
    return jax.nn.gelu(x, approximate=True)
def _silu(x):
    return jax.nn.silu(x)
def _sigmoid(x):
    return jax.nn.sigmoid(x)
def _layernorm(x, axis=-1, eps=1e-5):
    m = jnp.mean(x, axis=axis, keepdims=True)
    v = jnp.var(x, axis=axis, keepdims=True)
    return (x - m) / jnp.sqrt(v + eps)
def _scatter_add(tgt, idx, src, axis=0):
    return tgt.at[idx].add(src)
def _segment_sum(src, seg, n):
    return jax.ops.segment_sum(src, seg, n)
class _Rng:
    def __init__(self, key):
        self._k = key
    def _next(self):
        self._k, sub = jax.random.split(self._k)
        return sub
    def normal(self, shape):
        return jax.random.normal(self._next(), shape, dtype=jnp.bfloat16)
    def randint(self, lo, hi, shape):
        return jax.random.randint(self._next(), shape, lo, hi, dtype=jnp.int32)
    def uniform(self, shape, lo=0.0, hi=1.0):
        return jax.random.uniform(self._next(), shape, jnp.bfloat16, lo, hi)
    def permutation(self, n):
        return jax.random.permutation(self._next(), n)


kernel_name = 'standalone__seq2seq_rnn_t_joint__speech'

def setup_inputs():
    _rng = _Rng(jax.random.key(int.from_bytes(__import__("os").urandom(4), "little")))
    _w = (lambda a: (lambda t: t.astype(jnp.bfloat16) if jnp.issubdtype(t.dtype, jnp.floating) else t)(jnp.asarray(a)))
    B, T, D, K = 2, 16000, 256, 31
    U = 8
    sc = (1.0 / (K * D)) ** 0.5
    sd = (1.0 / D) ** 0.5
    return {
        "x": _w((lambda *s: _rng.normal(s) * 0.2)(B, T, D) * 0.5),
        "w1": _w((lambda *s: _rng.normal(s) * 1.6)(K, D, D) * sc),
        "w2": _w((lambda *s: _rng.normal(s) * 1.6)(K, D, D) * sc),
        "g": _w((lambda *s: _rng.normal(s) * 1.6)(B, U, D) * 0.5),
        "w_f": _w((lambda *s: _rng.normal(s) * 1.6)(D, D) * sd),
        "w_g": _w((lambda *s: _rng.normal(s) * 1.6)(D, D) * sd),
        "w_o": _w((lambda *s: _rng.normal(s) * 1.6)(D, D) * sd),
    }

def reference(x, w1, w2, g, w_f, w_g, w_o):
    B, T, D = x.shape
    K = w1.shape[0]
    pad = K // 2
    xp = jnp.pad(x, ((0,0),(pad,pad),(0,0)))
    h = jnp.zeros_like(x)
    for i in range(K):
        h = h + jnp.einsum("btc,cd->btd", xp[:, i:i+T, :], w1[i])
    h = _gelu(h)[:, ::2, :]
    T1 = h.shape[1]
    hp = jnp.pad(h, ((0,0),(pad,pad),(0,0)))
    f = jnp.zeros_like(h)
    for i in range(K):
        f = f + jnp.einsum("btc,cd->btd", hp[:, i:i+T1, :], w2[i])
    f = _gelu(f)[:, ::2, :]
    fe = jnp.einsum("btd,de->bte", f, w_f)
    ge = jnp.einsum("bud,de->bue", g, w_g)
    j = jnp.tanh(fe[:, :, None, :] + ge[:, None, :, :])
    return jnp.einsum("btud,dv->btuv", j, w_o)
```

```python
import numpy as np
import ml_dtypes
import jax
import jax.numpy as jnp
from jax import lax
import jax.experimental.pallas as pl
import jax.experimental.pallas.tpu as pltpu

NF = 128
L = 48
NK = 32
BF = jnp.bfloat16
F32 = jnp.float32
U32 = jnp.uint32

NPS = 172
SW = 260
MS = 340
TT = 800
NRING = 2
TS = 200
UA, UB, UC, UD = 32, 28, 4, 84
XA = 0


def _consts(ntaps):
    k = np.arange(NK)
    ph = lambda kk: 2 * np.pi * (kk + 0.5) / NF
    n = np.arange(NF)
    fx = np.concatenate([np.cos(np.outer(ph(k), n)), np.cos(np.outer(ph(63 - k), n)),
                         -np.sin(np.outer(ph(k), n)), np.sin(np.outer(ph(63 - k), n))])
    i1 = np.arange(32) + 1
    fw = np.concatenate([np.cos(np.outer(ph(k), i1)), np.cos(np.outer(ph(63 - k), i1)),
                         np.sin(np.outer(ph(k), i1)), -np.sin(np.outer(ph(63 - k), i1))])
    fw[:, ntaps:] = 0
    fw2 = np.concatenate([np.kron(fw, np.array([[1.0, 0.0]])), np.kron(fw, np.array([[0.0, 1.0]]))])
    th = 2 * np.pi * np.outer(np.r_[0:L:2, 1:L:2], k + 0.5) / 64
    gi = np.stack([np.cos(th), -np.sin(th)], -1).reshape(L, 2 * NK) / 64

    def c(a):
        u = a.astype(np.float32).astype(ml_dtypes.bfloat16).view(np.uint16).astype(np.uint32)
        return u[0::2] | (u[1::2] << 16)
    return c(fx), c(fw2), c(gi)


def _gelu(x):
    c = float(np.sqrt(2 / np.pi))
    inner = x * (c + (c * 0.044715) * (x * x))
    hx = 0.5 * x
    return hx + hx * jnp.tanh(inner)


def _pack(a, b):
    return pltpu.pack_elementwise([a, b], packed_dtype=BF)


def _dot(a, b):
    return jnp.dot(a, b, preferred_element_type=F32)


def _rows(ref, b, r, n):
    return jnp.concatenate([pltpu.bitcast(ref[b, ct, pl.ds(r, n), :], BF) for ct in range(2)], axis=1)


def _loop(name, n, f):
    with jax.named_scope("ph_" + name):
        lax.fori_loop(0, n, f, 0)


def _body(x_hbm, w1_hbm, w2_hbm, g_ref, wf_ref, wg_ref, wo_ref, fx_ref, fw_ref, gi_ref,
          out_hbm, xs, wb, what, xhat, yhat, fes, ges, ring, wsems, sems, osems):
    T = x_hbm.shape[1]
    KD = w1_hbm.shape[0]
    NA = 64 // UA
    NXC = 84 // UB
    XR = 4 * L * UB

    def wcopy(w, dt):
        return pltpu.make_async_copy(w.at[:, pl.ds(128 * dt, 128)],
                                     wb.bitcast(BF).at[pl.ds(8192 * dt, KD)], wsems.at[dt])

    def xcopies(c):
        b, i = divmod(c, NXC)
        lo, hi = (XR * i + 16 if i else 0), min(XR * (i + 1) + 16, T)
        return [pltpu.make_async_copy(x_hbm.at[b, pl.ds(lo, hi - lo), pl.ds(128 * ct, 128)],
                                      xs.bitcast(BF).at[b, ct, pl.ds(16 + lo, hi - lo)], sems.at[c, ct])
                for ct in range(2)]

    def xwhen(cond, c, start):
        if 0 <= c < 2 * NXC:
            @pl.when(cond)
            def _():
                for cp in xcopies(c):
                    cp.start() if start else cp.wait()
    wcopy(w1_hbm, 0).start()

    def zero_rows(r0, n):
        for b in range(2):
            for ct in range(2):
                xs[b, ct, pl.ds(r0, n), :] = jnp.zeros((n, 128), U32)
    for dt in range(2):
        wb[pl.ds(4096 * dt + KD // 2, 128), :] = jnp.zeros((128, 128), U32)
    zero_rows(0, 8)
    zero_rows(8 + T // 2, xs.shape[2] - 8 - T // 2)
    ges[...] = _dot(g_ref[...], wg_ref[...])

    def phase_a(first):
        def it(i, _):
            if first:
                @pl.when(i == NA)
                def _():
                    wcopy(w1_hbm, 1).wait()
                for c in range(2 * NA - XA):
                    xwhen(i == c + XA, c, True)
            dt = i // NA
            m0 = (i - dt * NA) * UA
            for u in range(UA):
                m = m0 + u
                s = jnp.concatenate(
                    [pltpu.bitcast(wb[pl.ds(4096 * dt + 64 * e + m, 32, stride=128), :], BF) for e in range(2)], axis=1)
                r = _dot(pltpu.bitcast(fw_ref[...], BF), s)
                c0, d0, c1, d1 = r[:64], r[64:128], r[128:192], r[192:]
                for v, zp in enumerate((_pack(c0, c1), _pack(d0 - c0, d1 - c1), _pack(c0 + d0, c1 + d1))):
                    for hf in range(2):
                        for e in range(2):
                            what[v * 2 + dt, pl.ds(hf * 128 + 64 * e + m, NK, stride=SW), :] = (
                                zp[32 * hf:32 * hf + 32, 128 * e:128 * e + 128])
            return 0
        _loop('A', 2 * NA, it)

    def phase_b(b, npairs, first):
        ub = UB if first else npairs

        def it(i, _):
            if first:
                for c in range(NXC):
                    xwhen(i == c, b * NXC + c, False)
                    xwhen(i == c, b * NXC + c + 2 * NA - XA, True)
            for u in range(ub):
                j = i * ub + u
                p = _dot(pltpu.bitcast(fx_ref[...], BF), _rows(xs, b, pl.multiple_of(j * 2 * L, 8), NF // 2))
                q = _dot(pltpu.bitcast(fx_ref[...], BF), _rows(xs, b, pl.multiple_of(j * 2 * L + L, 8), NF // 2))
                zs = (_pack(p[:64] + p[64:], q[:64] + q[64:]), _pack(p[:64], q[:64]), _pack(p[64:], q[64:]))
                for v, z in enumerate(zs):
                    for hf in range(2):
                        for ct in range(2):
                            xhat[v * 4 + hf * 2 + ct, pl.ds(b * npairs + j, NK, stride=NPS), :] = (
                                z[32 * hf:32 * hf + 32, 128 * ct:128 * ct + 128])
            return 0
        _loop('B', npairs // ub, it)

    def phase_c(npairs, uc):
        def it(i, _):
            for u in range(uc):
                k = i * uc + u
                ks = []
                for v in range(3):
                    a = jnp.concatenate(
                        [pltpu.bitcast(xhat[v * 4 + kt, pl.ds(k * NPS, npairs), :], BF) for kt in range(4)], axis=1)
                    w = jnp.concatenate(
                        [pltpu.bitcast(what[v * 2 + dt, pl.ds(k * SW, 256), :], BF) for dt in range(2)], axis=1)
                    ks.append(_dot(a, w))
                z = _pack(ks[0] - ks[2], ks[0] + ks[1])
                for dt in range(2):
                    yhat[dt, pl.ds(k * MS, 2 * npairs), :] = z[:, 128 * dt:128 * dt + 128]
            return 0
        _loop('C', NK // uc, it)

    def phase_d(nblk):
        per = nblk // UD

        def it(i, _):
            b = i // per
            for u in range(UD):
                m = i * UD + u
                s = jnp.concatenate(
                    [pltpu.bitcast(yhat[dt, pl.ds(m, NK, stride=MS), :], BF) for dt in range(2)], axis=1)
                y = _gelu(_dot(pltpu.bitcast(gi_ref[...], BF), s))
                z = _pack(y[:L // 2], y[L // 2:])
                r = pl.multiple_of(8 + (m - b * nblk) * (L // 2), 8)
                for ct in range(2):
                    xs[b, ct, pl.ds(r, L // 2), :] = z[:, 128 * ct:128 * ct + 128]
            return 0
        _loop('D', 2 * per, it)

    wcopy(w1_hbm, 0).wait()
    wcopy(w1_hbm, 1).start()
    phase_a(True)
    for b in range(2):
        phase_b(b, 84, True)
    for dt in range(2):
        wcopy(w2_hbm, dt).start()
    phase_c(168, UC)
    phase_d(168)
    zero_rows(8 + T // 4, 48)
    for dt in range(2):
        wcopy(w2_hbm, dt).wait()
    phase_a(False)
    for b in range(2):
        phase_b(b, 42, False)
    phase_c(84, 2 * UC)
    phase_d(84)

    nch = (T // 4) // TT

    def ocopy(c, slot, s):
        return pltpu.make_async_copy(ring.at[slot, pl.ds(s * 8, TS * 8)],
                                     out_hbm.at[pl.ds(c * (TT * 8) + s * 8, TS * 8)], osems.at[slot, s // TS])

    def joint(c, _):
        b = c // nch
        t0 = pl.multiple_of(8 + (c - b * nch) * (TT // 2), 8)
        slot = c % NRING

        @pl.when(c >= NRING)
        def _():
            for s in range(0, TT, TS):
                ocopy(c - NRING, slot, s).wait()
        fes[...] = _dot(_rows(xs, b, t0, TT // 2), wf_ref[...])
        ge = ges[pl.ds(pl.multiple_of(b * 8, 8), 8), :]
        for s in range(0, TT, TS):
            jt = jnp.concatenate([jnp.tanh(fes[pl.ds(t, 1), :] + ge) for t in range(s, s + TS)], axis=0)
            ring[slot, pl.ds(s * 8, TS * 8)] = _dot(jt.astype(BF), wo_ref[...]).astype(BF)
            ocopy(c, slot, s).start()
        return 0
    _loop('E', 2 * nch, joint)
    for c in range(2 * nch - NRING, 2 * nch):
        for s in range(0, TT, TS):
            ocopy(c, c % NRING, s).wait()


@jax.jit
def pallas_standalone__seq2seq_rnn_t_joint__speech_kernel(x, w1, w2, g, w_f, w_g, w_o):
    B, T, D = x.shape
    K = w1.shape[0]
    U = g.shape[1]
    assert (B, T, D, K, U) == (2, 16000, 256, 31, 8)
    fx, fw2, gi = _consts(K)
    hbm = pl.BlockSpec(memory_space=pl.ANY)
    vm = pl.BlockSpec(memory_space=pltpu.VMEM)
    out = pl.pallas_call(
        _body,
        out_shape=jax.ShapeDtypeStruct((B * (T // 4) * U, D), x.dtype),
        in_specs=[hbm, hbm, hbm] + [vm] * 7,
        out_specs=hbm,
        scratch_shapes=[
            pltpu.VMEM((2, 2, L * 167 + NF // 2, 128), U32),
            pltpu.VMEM((32 * D, 128), U32),
            pltpu.VMEM((6, NK * SW, 128), U32),
            pltpu.VMEM((12, NK * NPS, 128), U32),
            pltpu.VMEM((2, NK * MS, 128), U32),
            pltpu.VMEM((TT, D), F32),
            pltpu.VMEM((B * U, D), F32),
            pltpu.VMEM((NRING, TT * U, D), BF),
            pltpu.SemaphoreType.DMA((2,)),
            pltpu.SemaphoreType.DMA((2 * 84 // UB, 2)),
            pltpu.SemaphoreType.DMA((NRING, TT // TS)),
        ],
        compiler_params=pltpu.CompilerParams(vmem_limit_bytes=120 * 1024 * 1024),
    )(x, w1.reshape(K * D, D), w2.reshape(K * D, D), g.reshape(B * U, D), w_f, w_g, w_o, fx, fw2, gi)
    return out.reshape(B, T // 4, U, D)
```
